```python
import os as _os
_os.environ.setdefault("JAX_PLATFORMS", "cpu")
import jax
import jax.numpy as jnp

def _softmax(x, axis=-1):
    return jax.nn.softmax(x, axis=axis)
def _gelu(x):
    return jax.nn.gelu(x, approximate=True)
def _silu(x):
    return jax.nn.silu(x)
def _sigmoid(x):
    return jax.nn.sigmoid(x)
def _layernorm(x, axis=-1, eps=1e-5):
    m = jnp.mean(x, axis=axis, keepdims=True)
    v = jnp.var(x, axis=axis, keepdims=True)
    return (x - m) / jnp.sqrt(v + eps)
def _scatter_add(tgt, idx, src, axis=0):
    return tgt.at[idx].add(src)
def _segment_sum(src, seg, n):
    return jax.ops.segment_sum(src, seg, n)
class _Rng:
    def __init__(self, key):
        self._k = key
    def _next(self):
        self._k, sub = jax.random.split(self._k)
        return sub
    def normal(self, shape):
        return jax.random.normal(self._next(), shape, dtype=jnp.bfloat16)
    def randint(self, lo, hi, shape):
        return jax.random.randint(self._next(), shape, lo, hi, dtype=jnp.int32)
    def uniform(self, shape, lo=0.0, hi=1.0):
        return jax.random.uniform(self._next(), shape, jnp.bfloat16, lo, hi)
    def permutation(self, n):
        return jax.random.permutation(self._next(), n)


kernel_name = 'standalone__channel_attn_cbam__vision'

def setup_inputs():
    _rng = _Rng(jax.random.key(int.from_bytes(__import__("os").urandom(4), "little")))
    _w = (lambda a: (lambda t: t.astype(jnp.bfloat16) if jnp.issubdtype(t.dtype, jnp.floating) else t)(jnp.asarray(a)))
    H = W = 384
    C = 192
    r = max(C // 4, 1)
    return {
        "x": _w((lambda *s: _rng.normal(s) * 0.2)(1, H, W, C) + (lambda *s: _rng.normal(s) * 0.2)(1, 1, 1, C) * 2.0),
        "w1": _w((lambda *s: _rng.normal(s) * 0.2)(C, r)),
        "w2": _w((lambda *s: _rng.normal(s) * 0.2)(r, C)),
    }

def reference(x, w1, w2):
    B, H, W, C = x.shape
    xf = x.reshape(B, H * W, C)
    gap = jnp.mean(xf, 1)
    gmp = jnp.amax(xf, 1)
    h_a = gap @ w1
    h_a = h_a * (lambda x, dt: x.astype(dt))(h_a > 0, h_a.dtype)
    h_m = gmp @ w1
    h_m = h_m * (lambda x, dt: x.astype(dt))(h_m > 0, h_m.dtype)
    scale = _sigmoid(h_a @ w2 + h_m @ w2)
    return x * scale[:, None, None, :]
```

```python
import jax
import jax.numpy as jnp
import numpy as np
import jax.experimental.pallas as pl
import jax.experimental.pallas.tpu as pltpu

LANES, SUB = 128, 8
RS, RP, RD, RNS = 12, 128, 8, 1
WS, WP, WNS = 6, 96, 3


@jax.jit
def pallas_standalone__channel_attn_cbam__vision_kernel(
    x: jax.Array,
    w1: jax.Array,
    w2: jax.Array,
):
    B, H, W, C = x.shape
    R = w1.shape[1]
    CT, WT = C // SUB, W // LANES
    PER = CT * WT * SUB
    N = H * PER
    RT, WTR = N // RS, N // WS
    RG, WG = RT // RP, WTR // WP
    assert B == 1 and RG * RP == RT and WG * WP == WTR and RT % PER == 0 and WTR % PER == 0
    RA = int(np.lcm(RP, PER))
    WA = int(np.lcm(WP, PER))

    def kern(x_hbm, w1_hbm, w2_hbm, o_hbm, buf, asum, amax, sc, w1v, w2v, rsem, wsem):
        rbuf = buf.reshape(RS, RT, LANES)
        wbuf = buf.reshape(WS, WTR, LANES)

        def rd_start(g, slot):
            rows = pl.ds(pl.multiple_of(g * RP, 16), RP)
            for j in range(RS // RNS):
                idx = (pl.ds(j * RNS, RNS), rows)
                pltpu.make_async_copy(x_hbm.at[idx], rbuf.at[idx], rsem.at[slot]).start(priority=j % 2)

        def rd_wait(g, slot):
            v = rbuf.at[:, pl.ds(pl.multiple_of(g * RP, 16), RP)]
            pltpu.make_async_copy(v, v, rsem.at[slot]).wait()

        def reduce_step(g):
            a0 = pl.multiple_of((g % (RA // RP)) * RP, 16)
            r0 = pl.multiple_of(g * RP, 16)
            for v in range(RP // 16):
                ar = pl.ds(a0 + v * 16, 16)
                s = asum[ar, :]
                m = amax[ar, :]
                for j in range(RS):
                    t = rbuf[j, pl.ds(r0 + v * 16, 16), :].astype(jnp.float32)
                    s = s + t
                    m = jnp.maximum(m, t)
                asum[ar, :] = s
                amax[ar, :] = m

        for g in range(RD):
            rd_start(g, g)
        cw1 = pltpu.make_async_copy(w1_hbm, w1v, wsem)
        cw2 = pltpu.make_async_copy(w2_hbm, w2v, wsem)
        cw1.start()
        cw2.start()
        asum[...] = jnp.zeros(asum.shape, jnp.float32)
        amax[...] = jnp.full(amax.shape, -jnp.inf, jnp.float32)

        @pl.loop(0, RG - RD)
        def _(g):
            slot = g % RD
            rd_wait(g, slot)
            rd_start(g + RD, slot)
            reduce_step(g)

        cw1.wait()
        cw2.wait()
        w1f = w1v[...].astype(jnp.float32).T
        w2f = w2v[...].astype(jnp.float32).T

        @pl.loop(RG - RD, RG)
        def _(g):
            rd_wait(g, g % RD)
            reduce_step(g)

        def fold(ref, op):
            outs = []
            for ct in range(CT):
                acc = None
                for rep in range(RA // PER):
                    for wt in range(WT):
                        t = ref[pl.ds(rep * PER + (ct * WT + wt) * SUB, SUB), :]
                        acc = t if acc is None else op(acc, t)
                outs.append(acc)
            return jnp.concatenate(outs, axis=0)

        gap = jnp.sum(fold(asum, jnp.add), axis=1, keepdims=True) * np.float32(1.0 / (H * W))
        gmp = jnp.max(fold(amax, jnp.maximum), axis=1, keepdims=True)
        ha = jnp.sum(gap * w1f, axis=0, keepdims=True)
        hm = jnp.sum(gmp * w1f, axis=0, keepdims=True)
        ha = ha * (ha > 0).astype(jnp.float32)
        hm = hm * (hm > 0).astype(jnp.float32)
        z = jnp.sum((ha + hm) * w2f, axis=1, keepdims=True)
        scale = jax.nn.sigmoid(jnp.broadcast_to(z, (C, LANES)))
        for rep in range(WA // PER):
            for ct in range(CT):
                for wt in range(WT):
                    sc[pl.ds(rep * PER + (ct * WT + wt) * SUB, SUB), :] = scale[ct * SUB:(ct + 1) * SUB]

        @pl.loop(0, WG)
        def _(g):
            a0 = pl.multiple_of((g % (WA // WP)) * WP, 16)
            r0 = pl.multiple_of(g * WP, 16)
            for v in range(WP // 16):
                s = sc[pl.ds(a0 + v * 16, 16), :]
                for j in range(WS):
                    rr = pl.ds(r0 + v * 16, 16)
                    wbuf[j, rr, :] = (wbuf[j, rr, :].astype(jnp.float32) * s).astype(buf.dtype)
            for j in range(WS // WNS):
                idx = (pl.ds(j * WNS, WNS), pl.ds(r0, WP))
                pltpu.make_async_copy(wbuf.at[idx], o_hbm.at[idx], wsem).start(priority=j % 2)

        pltpu.make_async_copy(wbuf, o_hbm, wsem).wait()

    xt = jnp.transpose(x, (0, 1, 3, 2)).reshape(H, CT, SUB, WT, LANES)
    xt = jnp.transpose(xt, (0, 1, 3, 2, 4)).reshape(RS, RT, LANES)
    any_spec = pl.BlockSpec(memory_space=pl.ANY)
    o = pl.pallas_call(
        kern,
        in_specs=[any_spec] * 3,
        out_specs=any_spec,
        out_shape=jax.ShapeDtypeStruct((WS, WTR, LANES), x.dtype),
        scratch_shapes=[
            pltpu.VMEM((N, LANES), x.dtype),
            pltpu.VMEM((RA, LANES), jnp.float32),
            pltpu.VMEM((RA, LANES), jnp.float32),
            pltpu.VMEM((WA, LANES), jnp.float32),
            pltpu.VMEM((R, C), w1.dtype),
            pltpu.VMEM((R, C), w2.dtype),
            pltpu.SemaphoreType.DMA((RD,)),
            pltpu.SemaphoreType.DMA,
        ],
        compiler_params=pltpu.CompilerParams(vmem_limit_bytes=100 * 1024 * 1024),
    )(xt, w1.T, w2)
    o = o.reshape(H, CT, WT, SUB, LANES)
    o = jnp.transpose(o, (0, 1, 3, 2, 4)).reshape(B, H, C, W)
    return jnp.transpose(o, (0, 1, 3, 2))
```

```python
import functools

import jax
import jax.experimental.pallas as pl
import jax.experimental.pallas.tpu as pltpu
import jax.numpy as jnp
import numpy as np
from jax import lax

LANES = 128
TILE_ROWS = 8
UNIT_ROWS = 64
STREAM_ROWS = 4096
READ_UNITS = 2
WRITE_STREAMS = 6
READ_STEPS_IN_FLIGHT = 3
LAST_GROUP = 2


def _tree(op, values):
    while len(values) > 1:
        pairs = [values[i : i + 2] for i in range(0, len(values), 2)]
        values = [op(*p) if len(p) == 2 else p[0] for p in pairs]
    return values[0]


def _relu(h):
    return h * (h > 0).astype(h.dtype)


def _cbam_body(
    x_hbm, w1_hbm, w2_hbm, o_hbm,
    buf, sum_ref, max_ref, w1_raw, w2_raw, w1_ref, w2_ref,
    step_sems, tail_sems, sem,
    *, width, pixels,
):
    streams, stream_rows, _ = buf.shape
    channels, hidden = w1_ref.shape
    col_tiles = width // LANES
    unit_tiles = UNIT_ROWS // TILE_ROWS
    units = stream_rows // UNIT_ROWS
    steps = units // READ_UNITS
    half = streams // 2
    phases = channels * col_tiles // UNIT_ROWS
    blocks = streams // phases

    def channel_tile(phase, t):
        return (phase * unit_tiles + t) // col_tiles

    def stream_with(phase, q_mod):
        s = phase - q_mod
        return jnp.where(s < 0, s + phases, s)

    def rows(q, n=1):
        start = q * UNIT_ROWS
        if not isinstance(q, int):
            start = pl.multiple_of(start, UNIT_ROWS)
        return pl.ds(start, n * UNIT_ROWS)

    def read(s, step, read_sem):
        piece = (s, rows(step * READ_UNITS, READ_UNITS))
        return pltpu.make_async_copy(x_hbm.at[piece], buf.at[piece], read_sem)

    def write(s, q):
        return pltpu.make_async_copy(buf.at[s, rows(q)], o_hbm.at[s, rows(q)], sem)

    def pool(items):
        tiles = {}
        for phase, s, q in items:
            v = buf[s, rows(q)].astype(jnp.float32)
            for t in range(unit_tiles):
                tile = v[t * TILE_ROWS : (t + 1) * TILE_ROWS]
                tiles.setdefault(channel_tile(phase, t), []).append(tile)
        return [
            (ct, _tree(jnp.add, ts + [sum_ref[ct]]), _tree(jnp.maximum, ts + [max_ref[ct]]))
            for ct, ts in tiles.items()
        ]

    def step_sem(step):
        return step_sems.at[lax.rem(step, READ_STEPS_IN_FLIGHT)]

    def issue(step):
        @pl.loop(0, half)
        def _(j):
            read(2 * j, step, step_sem(step)).start(priority=0)
            read(2 * j + 1, step + 1, step_sem(step + 1)).start(priority=1)

    last = steps - 1
    groups = [[c + a * phases for a in range(blocks)] for c in range(phases)]
    groups[-1:] = [groups[-1][:-LAST_GROUP], groups[-1][-LAST_GROUP:]]
    tail = [(s, k) for k, group in enumerate(groups) for s in group]
    tail_high = tail[0 : half - 1 : 2]
    tail_low = [item for item in tail if item not in tail_high]

    def issue_tail(items, priority):
        for s, k in items:
            read(s, last, tail_sems.at[k]).start(priority=priority)

    for j in range(half):
        read(2 * j + 1, 0, step_sems.at[0]).start(priority=1)
    weight_copies = [
        pltpu.make_async_copy(w1_hbm, w1_raw, sem),
        pltpu.make_async_copy(w2_hbm, w2_raw, sem),
    ]
    for copy in weight_copies:
        copy.start()
    pl.loop(0, READ_STEPS_IN_FLIGHT - 1)(issue)
    sum_ref[...] = jnp.zeros(sum_ref.shape, jnp.float32)
    max_ref[...] = jnp.full(max_ref.shape, -jnp.inf, jnp.float32)
    for copy in weight_copies:
        copy.wait()
    w1_ref[...] = w1_raw[...].astype(jnp.float32).T
    w2_ref[...] = w2_raw[...].astype(jnp.float32).T

    @pl.loop(0, last)
    def _(step):
        q = step * READ_UNITS
        landed = buf.at[:, rows(q, READ_UNITS)]
        pltpu.make_async_copy(landed, landed, step_sem(step)).wait()

        ahead = step + READ_STEPS_IN_FLIGHT - 1
        pl.when(ahead < last - 1)(lambda: issue(ahead))

        @pl.when(ahead == last - 1)
        def _():
            slot = (last - 1) % READ_STEPS_IN_FLIGHT
            for j in range(half):
                read(2 * j, last - 1, step_sems.at[slot]).start(priority=0)
                issue_tail(tail_low[j : j + 1], 1)

        @pl.when(ahead == last)
        def _():
            for j in range(half):
                issue_tail(tail_high[j : j + 1], 0)
                issue_tail(tail_low[half + j : half + j + 1], 1)

        q_mod = lax.rem(q, phases)

        @pl.loop(0, blocks)
        def _(a):
            items = [
                (p, a * phases + stream_with(p - u, q_mod), q + u)
                for p in range(phases)
                for u in range(READ_UNITS)
            ]
            for ct, total, peak in pool(items):
                sum_ref[ct] = total
                max_ref[ct] = peak

    group_items = [
        [((s + q) % phases, s, q) for s in group for q in range(last * READ_UNITS, units)]
        for group in groups
    ]
    final_group = {
        channel_tile(phase, t): k
        for k, items in enumerate(group_items)
        for phase, _, _ in items
        for t in range(unit_tiles)
    }
    h_avg = h_max = jnp.zeros((TILE_ROWS, hidden), jnp.float32)
    for k, group in enumerate(groups):
        for s in group:
            read(s, last, tail_sems.at[k]).wait()
        avg_terms, max_terms = [h_avg], [h_max]
        for ct, total, peak in pool(group_items[k]):
            if final_group[ct] == k:
                w = w1_ref[pl.ds(ct * TILE_ROWS, TILE_ROWS), :]
                w_mean = w * np.float32(1.0 / pixels)
                avg_terms.append(jnp.sum(total, axis=1, keepdims=True) * w_mean)
                max_terms.append(jnp.max(peak, axis=1, keepdims=True) * w)
            else:
                sum_ref[ct] = total
                max_ref[ct] = peak
        h_avg, h_max = _tree(jnp.add, avg_terms), _tree(jnp.add, max_terms)

    h_avg = _relu(jnp.sum(h_avg, axis=0, keepdims=True))
    h_max = _relu(jnp.sum(h_max, axis=0, keepdims=True))
    h = h_avg + h_max
    scales = []
    for ct in range(channels // TILE_ROWS):
        w = w2_ref[pl.ds(ct * TILE_ROWS, TILE_ROWS), :]
        logit = jnp.sum(h * w, axis=1, keepdims=True)
        scales.append(jax.nn.sigmoid(jnp.broadcast_to(logit, (TILE_ROWS, LANES))))

    def rescale(items):
        results = []
        for phase, s, q in items:
            scale = [scales[channel_tile(phase, t)] for t in range(unit_tiles)]
            v = buf[s, rows(q)].astype(jnp.float32) * jnp.concatenate(scale, axis=0)
            results.append(v.astype(buf.dtype))
        for (_, s, q), v in zip(items, results):
            buf[s, rows(q)] = v

    def flush(i):
        s0 = lax.div(i, units) * WRITE_STREAMS
        write(pl.ds(s0, WRITE_STREAMS), lax.rem(i, units)).start()

    for s in range(phases):
        rescale([(s, s, 0)])
        if s < WRITE_STREAMS:
            write(s, 0).start()

    @pl.loop(1, blocks * units)
    def _(i):
        s0, q = lax.div(i, units) * phases, lax.rem(i, units)
        q_mod = lax.rem(q, phases)
        items = [(p, s0 + stream_with(p, q_mod), q) for p in range(phases)]
        for p in range(0, phases, 3):
            rescale(items[p : p + 3])
        flush(i)

    pl.loop(blocks * units, streams // WRITE_STREAMS * units)(flush)
    pltpu.make_async_copy(buf, o_hbm, sem).wait()


def _cbam_kernel(*refs, phases, **params):
    pl.run_scoped(
        functools.partial(_cbam_body, *refs, **params),
        pltpu.SemaphoreType.DMA((READ_STEPS_IN_FLIGHT,)),
        pltpu.SemaphoreType.DMA((phases + 1,)),
        pltpu.SemaphoreType.DMA(()),
    )


@jax.jit
def pallas_standalone__channel_attn_cbam__vision_kernel(
    x: jax.Array,
    w1: jax.Array,
    w2: jax.Array,
):
    batch, height, width, channels = x.shape
    hidden = w1.shape[1]
    row_tiles, col_tiles = channels // TILE_ROWS, width // LANES
    image_row = channels * col_tiles
    phases = image_row // UNIT_ROWS
    streams = height * image_row // STREAM_ROWS
    assert batch == 1 and channels % TILE_ROWS == 0 and width % LANES == 0
    assert image_row % UNIT_ROWS == 0 and height * image_row % STREAM_ROWS == 0
    assert STREAM_ROWS // UNIT_ROWS % phases == 1 and WRITE_STREAMS <= phases
    assert streams % phases == 0 and streams % WRITE_STREAMS == 0 and streams % 2 == 0
    view = (streams, STREAM_ROWS, LANES)

    tiles = jnp.transpose(x, (0, 1, 3, 2))
    tiles = tiles.reshape(height, row_tiles, TILE_ROWS, col_tiles, LANES)
    tiles = jnp.transpose(tiles, (0, 1, 3, 2, 4)).reshape(view)

    in_hbm = pl.BlockSpec(memory_space=pl.ANY)
    out = pl.pallas_call(
        functools.partial(_cbam_kernel, phases=phases, width=width, pixels=height * width),
        in_specs=[in_hbm, in_hbm, in_hbm],
        out_specs=in_hbm,
        out_shape=jax.ShapeDtypeStruct(view, x.dtype),
        scratch_shapes=[
            pltpu.VMEM(view, x.dtype),
            pltpu.VMEM((row_tiles, TILE_ROWS, LANES), jnp.float32),
            pltpu.VMEM((row_tiles, TILE_ROWS, LANES), jnp.float32),
            pltpu.VMEM((hidden, channels), w1.dtype),
            pltpu.VMEM((hidden, channels), w2.dtype),
            pltpu.VMEM((channels, hidden), jnp.float32),
            pltpu.VMEM((channels, hidden), jnp.float32),
        ],
        compiler_params=pltpu.CompilerParams(vmem_limit_bytes=100 * 1024 * 1024),
    )(tiles, w1.T, w2)

    out = out.reshape(height, row_tiles, col_tiles, TILE_ROWS, LANES)
    out = jnp.transpose(out, (0, 1, 3, 2, 4)).reshape(batch, height, channels, width)
    return jnp.transpose(out, (0, 1, 3, 2))
```

```python
import functools

import jax
import jax.experimental.pallas as pl
import jax.experimental.pallas.tpu as pltpu
import jax.numpy as jnp
import numpy as np
from jax import lax

LANES = 128
TILE_ROWS = 8
UNIT_ROWS = 64
STREAM_ROWS = 4096
READ_UNITS = 2
WRITE_STREAMS = 6
READ_STEPS_IN_FLIGHT = 3
LAST_GROUP = 2


def _tree(op, values):
    while len(values) > 1:
        pairs = [values[i : i + 2] for i in range(0, len(values), 2)]
        values = [op(*p) if len(p) == 2 else p[0] for p in pairs]
    return values[0]


def _relu(h):
    return h * (h > 0).astype(h.dtype)


def _cbam_body(
    x_hbm, w1_hbm, w2_hbm, o_hbm,
    buf, sum_ref, max_ref, w1_raw, w2_raw, w1_ref, w2_ref,
    step_sems, tail_sems, sem,
    *, width, pixels,
):
    streams, stream_rows, _ = buf.shape
    channels, hidden = w1_ref.shape
    row_tiles, col_tiles = channels // TILE_ROWS, width // LANES
    units = stream_rows // UNIT_ROWS
    steps = units // READ_UNITS
    half = streams // 2
    phases = channels * col_tiles // UNIT_ROWS
    blocks = streams // phases

    def channel_tiles(phase, n):
        starts = range(phase * UNIT_ROWS, (phase + n) * UNIT_ROWS, TILE_ROWS)
        return [r // (TILE_ROWS * col_tiles) % row_tiles for r in starts]

    def stream_with(block, phase, q):
        s = phase - lax.rem(q, phases)
        return block * phases + jnp.where(s < 0, s + phases, s)

    def rows(q, n=1):
        start = q * UNIT_ROWS
        if not isinstance(q, int):
            start = pl.multiple_of(start, UNIT_ROWS)
        return pl.ds(start, n * UNIT_ROWS)

    def read(s, step, read_sem):
        piece = (s, rows(step * READ_UNITS, READ_UNITS))
        return pltpu.make_async_copy(x_hbm.at[piece], buf.at[piece], read_sem)

    def write(first, n, q):
        unit = (pl.ds(first, n), rows(q))
        return pltpu.make_async_copy(buf.at[unit], o_hbm.at[unit], sem)

    def step_sem(step):
        return step_sems.at[lax.rem(step, READ_STEPS_IN_FLIGHT)]

    def issue(step):
        @pl.loop(0, half)
        def _(j):
            read(2 * j, step, step_sem(step)).start(priority=0)
            read(2 * j + 1, step + 1, step_sem(step + 1)).start(priority=1)

    last = steps - 1
    groups = [[c + a * phases for a in range(blocks)] for c in range(phases)]
    groups[-1:] = [groups[-1][:-LAST_GROUP], groups[-1][-LAST_GROUP:]]
    tail = [(s, k) for k, group in enumerate(groups) for s in group]
    tail_high = tail[0 : half - 1 : 2]
    tail_low = [item for item in tail if item not in tail_high]

    def issue_tail(items, priority):
        for s, k in items:
            read(s, last, tail_sems.at[k]).start(priority=priority)

    for j in range(half):
        read(2 * j + 1, 0, step_sems.at[0]).start(priority=1)
    weight_copies = [
        pltpu.make_async_copy(w1_hbm, w1_raw, sem),
        pltpu.make_async_copy(w2_hbm, w2_raw, sem),
    ]
    for copy in weight_copies:
        copy.start()
    pl.loop(0, READ_STEPS_IN_FLIGHT - 1)(issue)
    sum_ref[...] = jnp.zeros(sum_ref.shape, jnp.float32)
    max_ref[...] = jnp.full(max_ref.shape, -jnp.inf, jnp.float32)
    for copy in weight_copies:
        copy.wait()
    w1_ref[...] = w1_raw[...].astype(jnp.float32).T
    w2_ref[...] = w2_raw[...].astype(jnp.float32).T

    @pl.loop(0, last)
    def _(step):
        q = step * READ_UNITS
        landed = buf.at[:, rows(q, READ_UNITS)]
        pltpu.make_async_copy(landed, landed, step_sem(step)).wait()

        ahead = step + READ_STEPS_IN_FLIGHT - 1
        pl.when(ahead < last - 1)(lambda: issue(ahead))

        @pl.when(ahead == last - 1)
        def _():
            slot = (last - 1) % READ_STEPS_IN_FLIGHT
            for j in range(half):
                read(2 * j, last - 1, step_sems.at[slot]).start(priority=0)
                issue_tail(tail_low[j : j + 1], 1)

        @pl.when(ahead == last)
        def _():
            for j in range(half):
                issue_tail(tail_high[j : j + 1], 0)
                issue_tail(tail_low[half + j : half + j + 1], 1)

        @pl.loop(0, blocks)
        def _(block):
            order = [i * READ_UNITS % phases for i in range(phases)]
            pieces = [buf[stream_with(block, p, q), rows(q, READ_UNITS)] for p in order]
            v = jnp.concatenate(pieces, axis=0).astype(jnp.float32)
            v = v.reshape(READ_UNITS, row_tiles, col_tiles, TILE_ROWS, LANES)
            sum_ref[...] += jnp.sum(v, axis=(0, 2))
            max_ref[...] = jnp.maximum(max_ref[...], jnp.max(v, axis=(0, 2)))

    q = last * READ_UNITS
    group_tiles = [channel_tiles((group[0] + q) % phases, READ_UNITS) for group in groups]
    final_group = {ct: k for k, cts in enumerate(group_tiles) for ct in cts}
    h_avg = h_max = jnp.zeros((TILE_ROWS, hidden), jnp.float32)
    for k, group in enumerate(groups):
        for s in group:
            read(s, last, tail_sems.at[k]).wait()
        tiles = {}
        for s in group:
            v = buf[s, rows(q, READ_UNITS)].astype(jnp.float32)
            for t, ct in enumerate(group_tiles[k]):
                tiles.setdefault(ct, []).append(v[t * TILE_ROWS : (t + 1) * TILE_ROWS])
        avg_terms, max_terms = [h_avg], [h_max]
        for ct, new in tiles.items():
            total = _tree(jnp.add, new + [sum_ref[ct]])
            peak = _tree(jnp.maximum, new + [max_ref[ct]])
            if final_group[ct] == k:
                w = w1_ref[pl.ds(ct * TILE_ROWS, TILE_ROWS), :]
                w_mean = w * np.float32(1.0 / pixels)
                avg_terms.append(jnp.sum(total, axis=1, keepdims=True) * w_mean)
                max_terms.append(jnp.max(peak, axis=1, keepdims=True) * w)
            else:
                sum_ref[ct] = total
                max_ref[ct] = peak
        h_avg, h_max = _tree(jnp.add, avg_terms), _tree(jnp.add, max_terms)

    h_avg = _relu(jnp.sum(h_avg, axis=0, keepdims=True))
    h_max = _relu(jnp.sum(h_max, axis=0, keepdims=True))
    h = h_avg + h_max
    scales = []
    for ct in range(row_tiles):
        w = w2_ref[pl.ds(ct * TILE_ROWS, TILE_ROWS), :]
        logit = jnp.sum(h * w, axis=1, keepdims=True)
        scales.append(jax.nn.sigmoid(jnp.broadcast_to(logit, (TILE_ROWS, LANES))))

    def rescale(first, n, q, phase):
        scale = jnp.concatenate([scales[ct] for ct in channel_tiles(phase, n)], axis=0)
        unit = (pl.ds(first, n), rows(q))
        v = buf[unit].astype(jnp.float32) * scale.reshape(n, UNIT_ROWS, LANES)
        buf[unit] = v.astype(buf.dtype)

    for s in range(phases):
        rescale(s, 1, 0, s)
        write(s, 1, 0).start()

    @pl.loop(0, streams // WRITE_STREAMS)
    def _(i):
        @pl.loop(0, units - 1, step=phases)
        def _(q):
            for u in range(1, phases + 1):
                pl.when(i < blocks)(functools.partial(rescale, i * phases, phases, q + u, u))
                write(i * WRITE_STREAMS, WRITE_STREAMS, q + u).start()

    @pl.loop(1, blocks)
    def _(block):
        rescale(block * phases, phases, 0, 0)
        write(block * phases, phases, 0).start()

    pltpu.make_async_copy(buf, o_hbm, sem).wait()


def _cbam_kernel(*refs, phases, **params):
    pl.run_scoped(
        functools.partial(_cbam_body, *refs, **params),
        pltpu.SemaphoreType.DMA((READ_STEPS_IN_FLIGHT,)),
        pltpu.SemaphoreType.DMA((phases + 1,)),
        pltpu.SemaphoreType.DMA(()),
    )


@jax.jit
def pallas_standalone__channel_attn_cbam__vision_kernel(
    x: jax.Array,
    w1: jax.Array,
    w2: jax.Array,
):
    batch, height, width, channels = x.shape
    hidden = w1.shape[1]
    row_tiles, col_tiles = channels // TILE_ROWS, width // LANES
    image_row = channels * col_tiles
    phases = image_row // UNIT_ROWS
    streams = height * image_row // STREAM_ROWS
    assert batch == 1 and channels % TILE_ROWS == 0 and width % LANES == 0
    assert image_row % UNIT_ROWS == 0 and height * image_row % STREAM_ROWS == 0
    assert STREAM_ROWS // UNIT_ROWS % phases == 1 and WRITE_STREAMS <= phases
    assert np.gcd(READ_UNITS, phases) == 1 and streams // phases > LAST_GROUP
    assert streams % phases == 0 and streams % WRITE_STREAMS == 0 and streams % 2 == 0
    view = (streams, STREAM_ROWS, LANES)

    tiles = jnp.transpose(x, (0, 1, 3, 2))
    tiles = tiles.reshape(height, row_tiles, TILE_ROWS, col_tiles, LANES)
    tiles = jnp.transpose(tiles, (0, 1, 3, 2, 4)).reshape(view)

    in_hbm = pl.BlockSpec(memory_space=pl.ANY)
    out = pl.pallas_call(
        functools.partial(_cbam_kernel, phases=phases, width=width, pixels=height * width),
        in_specs=[in_hbm, in_hbm, in_hbm],
        out_specs=in_hbm,
        out_shape=jax.ShapeDtypeStruct(view, x.dtype),
        scratch_shapes=[
            pltpu.VMEM(view, x.dtype),
            pltpu.VMEM((row_tiles, TILE_ROWS, LANES), jnp.float32),
            pltpu.VMEM((row_tiles, TILE_ROWS, LANES), jnp.float32),
            pltpu.VMEM((hidden, channels), w1.dtype),
            pltpu.VMEM((hidden, channels), w2.dtype),
            pltpu.VMEM((channels, hidden), jnp.float32),
            pltpu.VMEM((channels, hidden), jnp.float32),
        ],
        compiler_params=pltpu.CompilerParams(vmem_limit_bytes=100 * 1024 * 1024),
    )(tiles, w1.T, w2)

    out = out.reshape(height, row_tiles, col_tiles, TILE_ROWS, LANES)
    out = jnp.transpose(out, (0, 1, 3, 2, 4)).reshape(batch, height, channels, width)
    return jnp.transpose(out, (0, 1, 3, 2))
```
